```python
import os as _os
_os.environ.setdefault("JAX_PLATFORMS", "cpu")
import jax
import jax.numpy as jnp

def _softmax(x, axis=-1):
    return jax.nn.softmax(x, axis=axis)
def _gelu(x):
    return jax.nn.gelu(x, approximate=True)
def _silu(x):
    return jax.nn.silu(x)
def _sigmoid(x):
    return jax.nn.sigmoid(x)
def _layernorm(x, axis=-1, eps=1e-5):
    m = jnp.mean(x, axis=axis, keepdims=True)
    v = jnp.var(x, axis=axis, keepdims=True)
    return (x - m) / jnp.sqrt(v + eps)
def _scatter_add(tgt, idx, src, axis=0):
    return tgt.at[idx].add(src)
def _segment_sum(src, seg, n):
    return jax.ops.segment_sum(src, seg, n)
class _Rng:
    def __init__(self, key):
        self._k = key
    def _next(self):
        self._k, sub = jax.random.split(self._k)
        return sub
    def normal(self, shape):
        return jax.random.normal(self._next(), shape, dtype=jnp.bfloat16)
    def randint(self, lo, hi, shape):
        return jax.random.randint(self._next(), shape, lo, hi, dtype=jnp.int32)
    def uniform(self, shape, lo=0.0, hi=1.0):
        return jax.random.uniform(self._next(), shape, jnp.bfloat16, lo, hi)
    def permutation(self, n):
        return jax.random.permutation(self._next(), n)


kernel_name = 'parallel_sum__ssm_conv_s5__geglu_ffn__prompt'

def setup_inputs():
    _rng = _Rng(jax.random.key(int.from_bytes(__import__("os").urandom(4), "little")))
    _w = (lambda a: (lambda t: t.astype(jnp.bfloat16) if jnp.issubdtype(t.dtype, jnp.floating) else t)(jnp.asarray(a)))
    def _A_setup():
        B, S, D = 1, 2048, 512
        P = D
        Lambda_re = -0.5 * jnp.exp((lambda *s: _rng.normal(s) * 0.8)(P))
        Lambda_im = (lambda *s: _rng.normal(s) * 0.8)(P) * 1.0
        B_re = (lambda *s: _rng.normal(s) * 0.8)(P, D) * (D ** -0.5)
        B_im = (lambda *s: _rng.normal(s) * 0.8)(P, D) * (D ** -0.5)
        C_re = (lambda *s: _rng.normal(s) * 0.8)(D, P) * (P ** -0.5)
        C_im = (lambda *s: _rng.normal(s) * 0.8)(D, P) * (P ** -0.5)
        log_dt = (lambda *s: _rng.normal(s) * 0.8)(P) * 0.3 - 2.0
        Dskip = (lambda *s: _rng.normal(s) * 0.8)(D)
        return {
            "x": _w((lambda *s: _rng.normal(s) * 0.05)(B, S, D)),
            "Lambda_re": _w(Lambda_re),
            "Lambda_im": _w(Lambda_im),
            "B_re": _w(B_re),
            "B_im": _w(B_im),
            "C_re": _w(C_re),
            "C_im": _w(C_im),
            "log_dt": _w(log_dt),
            "Dskip": _w(Dskip),
        }
    _A_in = _A_setup()

    def _B_setup():
        B, S, D, F = 1, 2048, 512, 1376
        return {
            "x": _w((lambda *s: _rng.normal(s) * 0.05)(B, S, D)),
            "w_gate": _w((lambda *s: _rng.normal(s) * 0.05)(D, F)),
            "w_up": _w((lambda *s: _rng.normal(s) * 0.05)(D, F)),
            "w_down": _w((lambda *s: _rng.normal(s) * 0.05)(F, D)),
        }
    _B_in = _B_setup()

    return {
        "A_x": _A_in["x"],
        "A_Lambda_re": _A_in["Lambda_re"],
        "A_Lambda_im": _A_in["Lambda_im"],
        "A_B_re": _A_in["B_re"],
        "A_B_im": _A_in["B_im"],
        "A_C_re": _A_in["C_re"],
        "A_C_im": _A_in["C_im"],
        "A_log_dt": _A_in["log_dt"],
        "A_Dskip": _A_in["Dskip"],
        "B_x": _B_in["x"],
        "B_w_gate": _B_in["w_gate"],
        "B_w_up": _B_in["w_up"],
        "B_w_down": _B_in["w_down"],
    }

def reference(A_x, A_Lambda_re, A_Lambda_im, A_B_re, A_B_im, A_C_re, A_C_im, A_log_dt, A_Dskip, B_x, B_w_gate, B_w_up, B_w_down):
    def _A_ref(x, Lambda_re, Lambda_im, B_re, B_im, C_re, C_im, log_dt, Dskip):
        Bsz, L, H = x.shape
        Lam = Lambda_re + 1j * Lambda_im
        Bmat = B_re + 1j * B_im
        Cmat = C_re + 1j * C_im
        dt = jnp.exp(log_dt)
        Lam_bar = jnp.exp(dt * Lam)
        B_bar = ((Lam_bar - 1.0) / Lam)[:, None] * Bmat
        Bu = jnp.einsum("bld,pd->blp", x + 0j, B_bar)
        h = jnp.zeros_like(Bu[:, 0, :])
        hs = []
        for t in range(L):
            h = Lam_bar[None, :] * h + Bu[:, t, :]
            hs.append(h)
        hseq = jnp.stack(hs, 1)
        y = 2.0 * jnp.einsum("blp,dp->bld", hseq, Cmat).real + x * Dskip[None, None, :]
        return y

    def _B_ref(x, w_gate, w_up, w_down):
        return (_gelu(x @ w_gate) * (x @ w_up)) @ w_down

    x = A_x
    xn = _layernorm(x, axis=-1)
    return x + _A_ref(xn, A_Lambda_re, A_Lambda_im, A_B_re, A_B_im, A_C_re, A_C_im, A_log_dt, A_Dskip) + _B_ref(xn, B_w_gate, B_w_up, B_w_down)
```

```python
import jax
import numpy as np
import jax, jax.numpy as jnp
from jax import lax
from jax.experimental import pallas as pl
from jax.experimental.pallas import tpu as pltpu

L, D, P, F = 2048, 512, 512, 1376
NT = (((1,), (1,)), ((), ()))
NN = (((1,), (0,)), ((), ()))
C0 = float(np.sqrt(2/np.pi)); C1 = float(np.sqrt(2/np.pi)*0.044715)
f32, bf16 = jnp.float32, jnp.bfloat16

def gelu_mul(g, u):
    inner = g * (C0 + C1 * (g*g))
    return (0.5 * g * u) * (1.0 + jnp.tanh(inner))

def cmul(ar, ai, br, bi):
    return ar*br - ai*bi, ar*bi + ai*br

import contextlib
def make(R=512, out_dtype=bf16, vmem_limit=100*2**20, order=0, scopes=False, flags=None):
    scope = (lambda n: jax.named_scope(n)) if scopes else (lambda n: contextlib.nullcontext())
    NB = L // R; T = R // 8
    PU = T + 1; PH = T//2 + 1
    logT = int(np.log2(T)); assert 2**logT == T

    def kernel(x_hbm, lre_hbm, lim_hbm, ldt_hbm, dsk_hbm, bre_hbm, bim_hbm, cre_hbm, cim_hbm, wg_hbm, wu_hbm, wd_hbm, out_hbm,
               xv, vecs, bre_v, bim_v, cre_v, cim_v, cp_v, wg_v, wu_v, wd_v, xn_s, base_s, us, hs, a_s, ov, sems):
        nsem = [0]
        def mk(src, dst):
            c = pltpu.make_async_copy(src, dst, sems.at[nsem[0]]); nsem[0] += 1
            c.start()
            return c
        cx = [None]*NB
        cx[0] = mk(x_hbm.at[pl.ds(0, R)], xv.at[0])
        cv = [mk(r, vecs.at[i]) for i, r in enumerate((lre_hbm, lim_hbm, ldt_hbm, dsk_hbm))]
        cbre = mk(bre_hbm, bre_v); cbim = mk(bim_hbm, bim_v)
        cwg = mk(wg_hbm, wg_v); cwu = mk(wu_hbm, wu_v)
        ccre = mk(cre_hbm, cre_v); ccim = mk(cim_hbm, cim_v)
        cwd = mk(wd_hbm, wd_v)
        for b in range(1, NB):
            cx[b] = mk(x_hbm.at[pl.ds(b*R, R)], xv.at[b])
        for c in cv: c.wait()
        lre = vecs[0].astype(f32); lim = vecs[1].astype(f32)
        dt = jnp.exp(vecs[2].astype(f32)).astype(bf16).astype(f32)
        dsk = vecs[3].astype(f32)
        dsk_row = jnp.concatenate([dsk[j:j+1] for j in range(4)], axis=1)
        mag = jnp.exp(dt*lre); ang = dt*lim
        ar4 = mag*jnp.cos(ang); ai4 = mag*jnp.sin(ang)
        den = lre*lre + lim*lim
        nr = ar4 - 1.0
        gr4 = (nr*lre + ai4*lim)/den; gi4 = (ai4*lre - nr*lim)/den
        pr, pi = ar4, ai4
        for _ in range(logT):
            pr, pi = cmul(pr, pi, pr, pi)
        p2r, p2i = cmul(pr, pi, pr, pi)
        p4r, p4i = cmul(p2r, p2i, p2r, p2i)
        bc = lambda v, j: jnp.broadcast_to(v[j:j+1], (8, 128))
        sub = lax.broadcasted_iota(jnp.int32, (8, 128), 0)

        def ln(b):
            cx[b].wait()
            xb = xv[b].astype(f32)
            m = jnp.mean(xb, axis=-1, keepdims=True)
            xc = xb - m
            v = jnp.mean(xc*xc, axis=-1, keepdims=True)
            xn = xc * lax.rsqrt(v + 1e-5)
            xn_s[b] = xn.astype(bf16)
            base_s[b] = xb + xn*dsk_row

        def umat(b):
            xn = xn_s[b]
            for part, w in ((0, bre_v), (4, bim_v)):
                if b == 0: (cbre if part == 0 else cbim).wait()
                u = lax.dot_general(xn, w[...], NT, preferred_element_type=f32)
                for j in range(4):
                    for s in range(8):
                        us[b, part+j, pl.ds(s*PU, T), :] = u[s*T:(s+1)*T, j*128:(j+1)*128]

        def scan(b, carry):
            ar = [bc(ar4, j) for j in range(4)]; ai = [bc(ai4, j) for j in range(4)]
            er = [None]*4; ei = [None]*4
            for t in range(T):
                for j in range(4):
                    ur = us[b, j, pl.ds(t, 8, stride=PU), :]
                    ui = us[b, 4+j, pl.ds(t, 8, stride=PU), :]
                    if t == 0:
                        er[j], ei[j] = ur, ui
                    else:
                        er[j], ei[j] = ar[j]*er[j] - ai[j]*ei[j] + ur, ar[j]*ei[j] + ai[j]*er[j] + ui
            hr = [None]*4; hi = [None]*4
            newc = []
            for j in range(4):
                if carry is None:
                    zr = jnp.where(sub == 0, 0.0, pltpu.roll(er[j], 1, 0))
                    zi = jnp.where(sub == 0, 0.0, pltpu.roll(ei[j], 1, 0))
                else:
                    zr = pltpu.roll(jnp.where(sub == 7, carry[j][0], er[j]), 1, 0)
                    zi = pltpu.roll(jnp.where(sub == 7, carry[j][1], ei[j]), 1, 0)
                for k, (qr, qi) in ((1, (pr, pi)), (2, (p2r, p2i)), (4, (p4r, p4i))):
                    mr = jnp.where(sub >= k, bc(qr, j), 0.0); mi = jnp.where(sub >= k, bc(qi, j), 0.0)
                    sr = pltpu.roll(zr, k, 0); si = pltpu.roll(zi, k, 0)
                    zr, zi = zr + (mr*sr - mi*si), zi + (mr*si + mi*sr)
                hr[j], hi[j] = zr, zi
                tr, ti = cmul(bc(pr, j), bc(pi, j), zr, zi)
                newc.append((er[j] + tr, ei[j] + ti))
            for tau in range(T//2):
                for j in range(4):
                    outs = []
                    for bb in range(2):
                        t = 2*tau + bb
                        ur = us[b, j, pl.ds(t, 8, stride=PU), :]
                        ui = us[b, 4+j, pl.ds(t, 8, stride=PU), :]
                        hr[j], hi[j] = ar[j]*hr[j] - ai[j]*hi[j] + ur, ar[j]*hi[j] + ai[j]*hr[j] + ui
                        outs.append((hr[j], hi[j]))
                    hs[b, j, pl.ds(tau, 8, stride=PH), :] = pltpu.pack_elementwise([outs[0][0], outs[1][0]], packed_dtype=bf16)
                    hs[b, 4+j, pl.ds(tau, 8, stride=PH), :] = pltpu.pack_elementwise([outs[0][1], outs[1][1]], packed_dtype=bf16)
            return newc

        def cprep():
            ccre.wait(); ccim.wait()
            for j in range(4):
                sl = slice(j*128, (j+1)*128)
                cr = cre_v[:, sl].astype(f32); ci = cim_v[:, sl].astype(f32)
                g_r = 2.0*gr4[j:j+1]; g_i = 2.0*gi4[j:j+1]
                cp_v[:, sl] = (cr*g_r - ci*g_i).astype(bf16)
                cp_v[:, pl.ds(512 + j*128, 128)] = (-(cr*g_i + ci*g_r)).astype(bf16)

        def ffn1(b):
            xn = xn_s[b]
            if b == 0: cwg.wait()
            g = lax.dot_general(xn, wg_v[...], NT, preferred_element_type=f32)
            if b == 0: cwu.wait()
            u = lax.dot_general(xn, wu_v[...], NT, preferred_element_type=f32)
            a_s[b] = gelu_mul(g, u).astype(bf16)

        def final(b):
            acc = base_s[b] + lax.dot_general(a_s[b], wd_v[...], NN, preferred_element_type=f32)
            H = jnp.concatenate([
                    jnp.concatenate([pltpu.bitcast(hs[b, jj, pl.ds(s*PH, T//2), :], bf16) for s in range(8)], axis=0)
                    for jj in range(8)], axis=1)
            acc = acc + lax.dot_general(H, cp_v[...], NT, preferred_element_type=f32)
            ov[b] = acc.astype(out_dtype)
            c = pltpu.make_async_copy(ov.at[b], out_hbm.at[pl.ds(b*R, R)], sems.at[nsem[0]]); nsem[0] += 1
            c.start()
            return c

        outs = []
        carry = None
        with scope("ln0"):
            ln(0)
        with scope("waitB"):
            pass
        for b in range(NB):
            with scope(f"U{b}"):
                umat(b)
            if b == 0:
                with scope("waitW"):
                    pass
            with scope(f"mid{b}"):
                if b + 1 < NB and order == 0:
                    ln(b+1)
                carry = scan(b, carry)
                ffn1(b)
                if b + 1 < NB and order == 1:
                    ln(b+1)
            if b + 1 < NB and order == 2 and b > 0:
                ln(b+1)
            if b == 0:
                with scope("cprep"):
                    cprep()
                    cwd.wait()
                    if order == 2: ln(1)
            with scope(f"fin{b}"):
                outs.append(final(b))
        with scope("tail"):
            for c in outs: c.wait()

    def f(A_x, A_Lambda_re, A_Lambda_im, A_B_re, A_B_im, A_C_re, A_C_im, A_log_dt, A_Dskip, B_x, B_w_gate, B_w_up, B_w_down):
        hbm = pl.BlockSpec(memory_space=pltpu.HBM)
        out = pl.pallas_call(kernel,
            out_shape=jax.ShapeDtypeStruct((L, D), out_dtype),
            in_specs=[hbm]*12, out_specs=hbm,
            scratch_shapes=[
                pltpu.VMEM((NB, R, D), bf16),
                pltpu.VMEM((4, 4, 128), bf16),
                pltpu.VMEM((P, D), bf16), pltpu.VMEM((P, D), bf16),
                pltpu.VMEM((D, P), bf16), pltpu.VMEM((D, P), bf16),
                pltpu.VMEM((D, 2*P), bf16),
                pltpu.VMEM((F, D), bf16), pltpu.VMEM((F, D), bf16), pltpu.VMEM((F, D), bf16),
                pltpu.VMEM((NB, R, D), bf16),
                pltpu.VMEM((NB, R, D), f32),
                pltpu.VMEM((NB, 8, 8*PU, 128), f32),
                pltpu.VMEM((NB, 8, 8*PH, 128), jnp.uint32),
                pltpu.VMEM((NB, R, F), bf16),
                pltpu.VMEM((NB, R, D), out_dtype),
                pltpu.SemaphoreType.DMA((32,)),
            ],
            compiler_params=pltpu.CompilerParams(vmem_limit_bytes=vmem_limit, flags=flags),
            name="ssm_ffn",
        )(A_x.reshape(L, D), A_Lambda_re.reshape(4,128), A_Lambda_im.reshape(4,128), A_log_dt.reshape(4,128), A_Dskip.reshape(4,128),
          A_B_re, A_B_im, A_C_re, A_C_im, B_w_gate.T, B_w_up.T, B_w_down)
        return out.reshape(1, L, D)
    return f


_impl = make(R=512, order=2)


@jax.jit
def pallas_parallel_sum__ssm_conv_s5__geglu_ffn__prompt_kernel(
    A_x, A_Lambda_re, A_Lambda_im, A_B_re, A_B_im, A_C_re, A_C_im, A_log_dt, A_Dskip,
    B_x, B_w_gate, B_w_up, B_w_down,
):
    return _impl(A_x, A_Lambda_re, A_Lambda_im, A_B_re, A_B_im, A_C_re, A_C_im, A_log_dt, A_Dskip,
                 B_x, B_w_gate, B_w_up, B_w_down)
```

```python
import jax
import contextlib
import numpy as np
import jax
import jax.numpy as jnp
from jax import lax
from jax.experimental import pallas as pl
from jax.experimental.pallas import tpu as pltpu

L, D, P, F = 2048, 512, 512, 1376
NT = (((1,), (1,)), ((), ()))
NN = (((1,), (0,)), ((), ()))
C0 = float(np.sqrt(2/np.pi)); C1 = float(np.sqrt(2/np.pi)*0.044715)
f32, bf16, u32 = jnp.float32, jnp.bfloat16, jnp.uint32


def b16(w):
    return pltpu.bitcast(w, bf16)


def w32(v):
    return pltpu.bitcast(v, u32)


def gelu_mul(g, u):
    inner = g * (C0 + C1 * (g*g))
    return (0.5 * g * u) * (1.0 + jnp.tanh(inner))


def cmul(ar, ai, br, bi):
    return ar*br - ai*bi, ar*bi + ai*br


def make(R=512, vmem_limit=100*2**20, scopes=False, flags=None, nx0=2, m0=2, nb=2, gch=(256, 256, 384, 480),
         nsplit=4, cch=32, lnch=32, dsc=False, sblk=-1, order=0, nrun=4):
    NB = L // R; T = R // 8
    PU = T + 1; PH = T//2 + 1
    logT = int(np.log2(T)); assert 2**logT == T
    assert sum(gch) == F
    scope = (lambda n: jax.named_scope(n)) if scopes else (lambda n: contextlib.nullcontext())
    def sc(n, b):
        return jax.named_scope(n) if b == sblk else contextlib.nullcontext()
    NSEM = 1 + nx0 + nb + 1 + len(gch) + 1 + 1 + 1 + 1

    def kernel(x_hbm, lre_hbm, lim_hbm, ldt_hbm, dsk_hbm, bre_hbm, bim_hbm, cre_hbm, cim_hbm, wg_hbm, wu_hbm, wd_hbm, out_hbm,
               xv, vecs, bre_v, bim_v, cre_v, cim_v, cp_v, wg_v, wu_v, wd_v, xn_s, base_s, us, hs, a_s, ov, sems):
        nsem = [0]
        def newsem():
            nsem[0] += 1
            return sems.at[nsem[0]-1]
        class W:
            def __init__(self, cs, name): self.cs = cs; self.name = name
            def wait(self):
                with scope("w_" + self.name):
                    for c in self.cs: c.wait()
        def mk(pairs, name):
            sem = newsem()
            cs = [pltpu.make_async_copy(s_, d_, sem) for s_, d_ in pairs]
            for c in cs: c.start()
            return W(cs, name)
        R0 = R // nx0
        x_hbm = x_hbm.bitcast(u32)
        bre_hbm, bim_hbm, cre_hbm, cim_hbm, wg_hbm, wu_hbm, wd_hbm = [r.bitcast(u32) for r in (bre_hbm, bim_hbm, cre_hbm, cim_hbm, wg_hbm, wu_hbm, wd_hbm)]
        PB = P // nb // 2
        x0p = lambda i: mk([(x_hbm.at[pl.ds(i*R0//2, R0//2)], xv.at[0, pl.ds(i*R0//2, R0//2)])], f"x0_{i}")
        brep = lambda i: mk([(bre_hbm.at[pl.ds(i*PB, PB)], bre_v.at[pl.ds(i*PB, PB)])], f"bre{i}")
        cx0 = [None]*nx0; cbre = [None]*nb
        cx0[0] = x0p(0)
        cv = mk([(r, vecs.at[i]) for i, r in enumerate((lre_hbm, lim_hbm, ldt_hbm, dsk_hbm))], "vec")
        if order == 0:
            cbre[0] = brep(0)
            for i in range(1, nx0): cx0[i] = x0p(i)
            for i in range(1, nb): cbre[i] = brep(i)
        elif order == 1:
            for i in range(1, nx0): cx0[i] = x0p(i)
            for i in range(nb): cbre[i] = brep(i)
        elif order == 2:
            for i in range(nb): cbre[i] = brep(i)
            for i in range(1, nx0): cx0[i] = x0p(i)
        cbim = mk([(bim_hbm, bim_v)], "bim")
        goff = [0]
        for g_ in gch: goff.append(goff[-1] + g_)
        cwg = [mk([(wg_hbm.at[pl.ds(goff[i]//2, gch[i]//2)], wg_v.at[pl.ds(goff[i]//2, gch[i]//2)])], f"wg{i}") for i in range(len(gch))]
        cwu = mk([(wu_hbm, wu_v)], "wu")
        cc = mk([(cre_hbm, cre_v), (cim_hbm, cim_v)], "c")
        cwd = mk([(wd_hbm, wd_v)] + [(x_hbm.at[pl.ds(b*R//2, R//2)], xv.at[b]) for b in range(1, NB)], "wd")
        osem = newsem()
        assert nsem[0] == NSEM, (nsem, NSEM)

        cv.wait()
        lre = vecs[0].astype(f32); lim = vecs[1].astype(f32)
        dt = jnp.exp(vecs[2].astype(f32)).astype(bf16).astype(f32)
        dsk = vecs[3].astype(f32)
        dsk_row = jnp.concatenate([dsk[j:j+1] for j in range(4)], axis=1)
        mag = jnp.exp(dt*lre); ang = dt*lim
        ar4 = mag*jnp.cos(ang); ai4 = mag*jnp.sin(ang)
        den = lre*lre + lim*lim
        nr = ar4 - 1.0
        gr4 = (nr*lre + ai4*lim)/den; gi4 = (ai4*lre - nr*lim)/den
        pr, pi = ar4, ai4
        for _ in range(logT):
            pr, pi = cmul(pr, pi, pr, pi)
        p2r, p2i = cmul(pr, pi, pr, pi)
        p4r, p4i = cmul(p2r, p2i, p2r, p2i)
        bc = lambda v, j: jnp.broadcast_to(v[j:j+1], (8, 128))
        sub = lax.broadcasted_iota(jnp.int32, (8, 128), 0)

        def ln_rows(b, r0, n):
            xb = b16(xv[b, pl.ds(r0//2, n//2), :]).astype(f32)
            m = jnp.mean(xb, axis=-1, keepdims=True)
            xc = xb - m
            v = jnp.mean(xc*xc, axis=-1, keepdims=True)
            xn = xc * lax.rsqrt(v + 1e-5)
            xn_s[b, pl.ds(r0, n), :] = xn.astype(bf16)
            base_s[b, pl.ds(r0, n), :] = xb + xn*dsk_row
        def ln(b, r0=0, n=R):
            for r in range(r0, r0+n, lnch):
                ln_rows(b, r, lnch)

        def ustore(b, part, u, j0, r0):
            nr_, nc = u.shape
            for j in range(nc // 128):
                for s in range(8):
                    lo = max(s*T, r0); hi = min((s+1)*T, r0 + nr_)
                    if hi > lo:
                        us[b, part+j0+j, pl.ds(s*PU + lo - s*T, hi - lo), :] = u[lo-r0:hi-r0, j*128:(j+1)*128]
        def umat(b):
            xn = xn_s[b]
            for part, w in ((0, bre_v), (4, bim_v)):
                u = lax.dot_general(xn, b16(w[...]), NT, preferred_element_type=f32)
                ustore(b, part, u, 0, 0)
        def block0_head():
            M0 = R // m0
            done = [False]*nx0
            def need_rows(r1):
                for i in range(nx0):
                    if i*R0 < r1 and not done[i]:
                        cx0[i].wait(); ln(0, i*R0, R0); done[i] = True
            for h in range(m0):
                need_rows((h+1)*M0)
                xn = xn_s[0, pl.ds(h*M0, M0), :]
                for i in range(nb):
                    if h == 0: cbre[i].wait()
                    u = lax.dot_general(xn, b16(bre_v[pl.ds(i*PB, PB), :]), NT, preferred_element_type=f32)
                    ustore(0, 0, u, i*(4//nb), h*M0)
            cbim.wait()
            xn = xn_s[0]
            u = lax.dot_general(xn, b16(bim_v[...]), NT, preferred_element_type=f32)
            ustore(0, 4, u, 0, 0)

        def scan(b, carry):
            ar = [bc(ar4, j) for j in range(4)]; ai = [bc(ai4, j) for j in range(4)]
            er = [None]*4; ei = [None]*4
            for t in range(T):
                for j in range(4):
                    ur = us[b, j, pl.ds(t, 8, stride=PU), :]
                    ui = us[b, 4+j, pl.ds(t, 8, stride=PU), :]
                    if t == 0:
                        er[j], ei[j] = ur, ui
                    else:
                        er[j], ei[j] = ar[j]*er[j] - ai[j]*ei[j] + ur, ar[j]*ei[j] + ai[j]*er[j] + ui
            hr = [None]*4; hi = [None]*4
            newc = []
            for j in range(4):
                if carry is None:
                    zr = jnp.where(sub == 0, 0.0, pltpu.roll(er[j], 1, 0))
                    zi = jnp.where(sub == 0, 0.0, pltpu.roll(ei[j], 1, 0))
                else:
                    zr = pltpu.roll(jnp.where(sub == 7, carry[j][0], er[j]), 1, 0)
                    zi = pltpu.roll(jnp.where(sub == 7, carry[j][1], ei[j]), 1, 0)
                for k, (qr, qi) in ((1, (pr, pi)), (2, (p2r, p2i)), (4, (p4r, p4i))):
                    mr = jnp.where(sub >= k, bc(qr, j), 0.0); mi = jnp.where(sub >= k, bc(qi, j), 0.0)
                    sr = pltpu.roll(zr, k, 0); si = pltpu.roll(zi, k, 0)
                    zr, zi = zr + (mr*sr - mi*si), zi + (mr*si + mi*sr)
                hr[j], hi[j] = zr, zi
                tr, ti = cmul(bc(pr, j), bc(pi, j), zr, zi)
                newc.append((er[j] + tr, ei[j] + ti))
            for tau in range(T//2):
                for j in range(4):
                    outs = []
                    for bb in range(2):
                        t = 2*tau + bb
                        ur = us[b, j, pl.ds(t, 8, stride=PU), :]
                        ui = us[b, 4+j, pl.ds(t, 8, stride=PU), :]
                        hr[j], hi[j] = ar[j]*hr[j] - ai[j]*hi[j] + ur, ar[j]*hi[j] + ai[j]*hr[j] + ui
                        outs.append((hr[j], hi[j]))
                    hs[b, j, pl.ds(tau, 8, stride=PH), :] = pltpu.pack_elementwise([outs[0][0], outs[1][0]], packed_dtype=bf16)
                    hs[b, 4+j, pl.ds(tau, 8, stride=PH), :] = pltpu.pack_elementwise([outs[0][1], outs[1][1]], packed_dtype=bf16)
            return newc

        def cprep():
            CH = cch
            for j in range(4):
                sl = slice(j*128, (j+1)*128)
                g_r = 2.0*gr4[j:j+1]; g_i = 2.0*gi4[j:j+1]
                ng_r = -g_r; ng_i = -g_i
                for r in range(0, D//2, CH//2):
                    cr = b16(cre_v[pl.ds(r, CH//2), sl]).astype(f32); ci = b16(cim_v[pl.ds(r, CH//2), sl]).astype(f32)
                    cp_v[pl.ds(r, CH//2), sl] = w32((cr*g_r - ci*g_i).astype(bf16))
                    cp_v[pl.ds(r, CH//2), pl.ds(512 + j*128, 128)] = w32((cr*ng_i + ci*ng_r).astype(bf16))

        def ffn1(b):
            xn = xn_s[b]
            with sc("gate", b):
                if b == 0:
                    gs = []
                    for i in range(len(gch)):
                        cwg[i].wait()
                        gs.append(lax.dot_general(xn, b16(wg_v[pl.ds(goff[i]//2, gch[i]//2), :]), NT, preferred_element_type=f32))
                    g = jnp.concatenate(gs, axis=1) if len(gs) > 1 else gs[0]
                    cwu.wait(); cc.wait()
                else:
                    g = lax.dot_general(xn, b16(wg_v[...]), NT, preferred_element_type=f32)
            with sc("up", b):
                u = lax.dot_general(xn, b16(wu_v[...]), NT, preferred_element_type=f32)
                a_s[b] = gelu_mul(g, u).astype(bf16)
            if b == 0:
                cprep()

        def final(b):
            with sc("down", b):
                acc = base_s[b] + lax.dot_general(a_s[b], b16(wd_v[...]), NN, preferred_element_type=f32)
            cs = []
            with sc("C", b):
                H = jnp.concatenate([
                        jnp.concatenate([pltpu.bitcast(hs[b, jj, pl.ds(s*PH, T//2), :], bf16) for s in range(8)], axis=0)
                        for jj in range(8)], axis=1)
                n = nsplit if b == nrun-1 else 1
                Wn = D // n
                for i in range(n):
                    a2 = acc[:, i*Wn:(i+1)*Wn] + lax.dot_general(H, b16(cp_v[pl.ds(i*Wn//2, Wn//2), :]), NT, preferred_element_type=f32)
                    ov[b, :, pl.ds(i*Wn, Wn)] = a2.astype(bf16)
                    c = pltpu.make_async_copy(ov.at[b, :, pl.ds(i*Wn, Wn)], out_hbm.at[pl.ds(b*R, R), pl.ds(i*Wn, Wn)], osem)
                    c.start(); cs.append(c)
            return cs

        outs = []
        carry = None
        for b in range(nrun):
            with sc("U", b):
                if b == 0: block0_head()
                else: umat(b)
            carry = scan(b, carry)
            ffn1(b)
            if b == 0:
                cwd.wait()
            if b + 1 < nrun: ln(b+1)
            outs += final(b)
        with scope("tail"):
            for c in outs: c.wait()

    def f(A_x, A_Lambda_re, A_Lambda_im, A_B_re, A_B_im, A_C_re, A_C_im, A_log_dt, A_Dskip, B_x, B_w_gate, B_w_up, B_w_down):
        hbm = pl.BlockSpec(memory_space=pltpu.HBM)
        out = pl.pallas_call(kernel,
            out_shape=jax.ShapeDtypeStruct((L, D), bf16),
            in_specs=[hbm]*12, out_specs=hbm,
            scratch_shapes=[
                pltpu.VMEM((NB, R//2, D), u32),
                pltpu.VMEM((4, 4, 128), bf16),
                pltpu.VMEM((P//2, D), u32), pltpu.VMEM((P//2, D), u32),
                pltpu.VMEM((D//2, P), u32), pltpu.VMEM((D//2, P), u32),
                pltpu.VMEM((D//2, 2*P), u32),
                pltpu.VMEM((F//2, D), u32), pltpu.VMEM((F//2, D), u32), pltpu.VMEM((F//2, D), u32),
                pltpu.VMEM((NB, R, D), bf16),
                pltpu.VMEM((NB, R, D), f32),
                pltpu.VMEM((NB, 8, 8*PU, 128), f32),
                pltpu.VMEM((NB, 8, 8*PH, 128), u32),
                pltpu.VMEM((NB, R, F), bf16),
                pltpu.VMEM((NB, R, D), bf16),
                pltpu.SemaphoreType.DMA((NSEM,)),
            ],
            compiler_params=pltpu.CompilerParams(vmem_limit_bytes=vmem_limit, flags=flags, disable_semaphore_checks=dsc),
            name="ssm_ffn",
        )(A_x.reshape(L, D), A_Lambda_re.reshape(4,128), A_Lambda_im.reshape(4,128), A_log_dt.reshape(4,128), A_Dskip.reshape(4,128),
          A_B_re, A_B_im, A_C_re, A_C_im, B_w_gate.T, B_w_up.T, B_w_down)
        return out.reshape(1, L, D)
    return f


_impl = make(nx0=1, m0=1, nb=1, flags={'XLA_TPU_RESCHEDULE_DMA_DONES': True})


@jax.jit
def pallas_parallel_sum__ssm_conv_s5__geglu_ffn__prompt_kernel(
    A_x, A_Lambda_re, A_Lambda_im, A_B_re, A_B_im, A_C_re, A_C_im, A_log_dt, A_Dskip,
    B_x, B_w_gate, B_w_up, B_w_down,
):
    return _impl(A_x, A_Lambda_re, A_Lambda_im, A_B_re, A_B_im, A_C_re, A_C_im, A_log_dt, A_Dskip,
                 B_x, B_w_gate, B_w_up, B_w_down)
```

```python
import jax
import contextlib
import numpy as np
import jax
import jax.numpy as jnp
from jax import lax
from jax.experimental import pallas as pl
from jax.experimental.pallas import tpu as pltpu

L, D, P, F = 2048, 512, 512, 1376
NT = (((1,), (1,)), ((), ()))
NN = (((1,), (0,)), ((), ()))
C0 = float(np.sqrt(2/np.pi)); C1 = float(np.sqrt(2/np.pi)*0.044715)
f32, bf16, u32 = jnp.float32, jnp.bfloat16, jnp.uint32


def b16(w):
    return pltpu.bitcast(w, bf16)


def w32(v):
    return pltpu.bitcast(v, u32)


def gelu_mul(g, u):
    inner = g * (C0 + C1 * (g*g))
    return (0.5 * g * u) * (1.0 + jnp.tanh(inner))


def dep0(v):
    z = jnp.minimum(pltpu.bitcast(v, jnp.int32) & 1, 0)
    return pltpu.bitcast(z, f32)


def cmul(ar, ai, br, bi):
    return ar*br - ai*bi, ar*bi + ai*br


def make(R=512, vmem_limit=100*2**20, scopes=False, flags=None, nx0=2, m0=2, nb=2, gch=(256, 256, 384, 480),
         nsplit=4, cch=32, lnch=32, dsc=False, sblk=-1, order=0, nrun=4, pace=(0,1,2,3,4), pace2=(5,6,7,8,9,10), lnd=True, prow=0, ablate='', cuts=(), hdep=True):
    NB = L // R; T = R // 8
    PU = T + 1; PH = T//2 + 1
    logT = int(np.log2(T)); assert 2**logT == T
    assert sum(gch) == F
    scope = (lambda n: jax.named_scope(n)) if scopes else (lambda n: contextlib.nullcontext())
    cur = [None]
    class sc:
        def __init__(self, n, b):
            if (n, b) in cuts:
                if cur[0] is not None: cur[0].__exit__(None, None, None)
                cur[0] = jax.named_scope(f"{n}{b}"); cur[0].__enter__()
        def __enter__(self): return self
        def __exit__(self, *a): return False
    NSEM = 1 + nx0 + nb + 1 + len(gch) + 1 + 1 + 1 + (NB - 1) + 1

    def kernel(x_hbm, lre_hbm, lim_hbm, ldt_hbm, dsk_hbm, bre_hbm, bim_hbm, cre_hbm, cim_hbm, wg_hbm, wu_hbm, wd_hbm, out_hbm,
               xv, vecs, bre_v, bim_v, cre_v, cim_v, cp_v, wg_v, wu_v, wd_v, xn_s, base_s, us, hs, a_s, ov, sems):
        nsem = [0]
        def newsem():
            nsem[0] += 1
            return sems.at[nsem[0]-1]
        class W:
            def __init__(self, cs, name): self.cs = cs; self.name = name
            def wait(self):
                with scope("w_" + self.name):
                    for c in self.cs: c.wait()
        def mk(pairs, name):
            sem = newsem()
            cs = [pltpu.make_async_copy(s_, d_, sem) for s_, d_ in pairs]
            for c in cs: c.start()
            return W(cs, name)
        R0 = R // nx0
        x_hbm = x_hbm.bitcast(u32)
        bre_hbm, bim_hbm, cre_hbm, cim_hbm, wg_hbm, wu_hbm, wd_hbm = [r.bitcast(u32) for r in (bre_hbm, bim_hbm, cre_hbm, cim_hbm, wg_hbm, wu_hbm, wd_hbm)]
        PB = P // nb // 2
        x0p = lambda i: mk([(x_hbm.at[pl.ds(i*R0//2, R0//2)], xv.at[0, pl.ds(i*R0//2, R0//2)])], f"x0_{i}")
        brep = lambda i: mk([(bre_hbm.at[pl.ds(i*PB, PB)], bre_v.at[pl.ds(i*PB, PB)])], f"bre{i}")
        cx0 = [None]*nx0; cbre = [None]*nb
        if isinstance(order, str):
            cv = None
            for tok in order.split():
                if tok[0] == 'x': cx0[int(tok[1:])] = x0p(int(tok[1:]))
                elif tok[0] == 'b': cbre[int(tok[1:])] = brep(int(tok[1:]))
                else: cv = mk([(r, vecs.at[i]) for i, r in enumerate((lre_hbm, lim_hbm, ldt_hbm, dsk_hbm))], "vec")
            assert all(c is not None for c in cx0 + cbre + [cv])
        else:
            cx0[0] = x0p(0)
            cv = mk([(r, vecs.at[i]) for i, r in enumerate((lre_hbm, lim_hbm, ldt_hbm, dsk_hbm))], "vec")
            if order == 0:
                cbre[0] = brep(0)
                for i in range(1, nx0): cx0[i] = x0p(i)
                for i in range(1, nb): cbre[i] = brep(i)
            elif order == 1:
                for i in range(1, nx0): cx0[i] = x0p(i)
                for i in range(nb): cbre[i] = brep(i)
            elif order == 2:
                for i in range(nb): cbre[i] = brep(i)
                for i in range(1, nx0): cx0[i] = x0p(i)
        cbim = mk([(bim_hbm, bim_v)], "bim")
        goff = [0]
        for g_ in gch: goff.append(goff[-1] + g_)
        cwg = [mk([(wg_hbm.at[pl.ds(goff[i]//2, gch[i]//2)], wg_v.at[pl.ds(goff[i]//2, gch[i]//2)])], f"wg{i}") for i in range(len(gch))]
        cwu = mk([(wu_hbm, wu_v)], "wu")
        cwd = mk([(wd_hbm, wd_v)], "wd")
        cc = mk([(cre_hbm, cre_v), (cim_hbm, cim_v)], "c")
        cx = [None] + [mk([(x_hbm.at[pl.ds(b*R//2, R//2)], xv.at[b])], f"x{b}") for b in range(1, NB)]
        osem = newsem()
        assert nsem[0] == NSEM, (nsem, NSEM)

        cv.wait()
        lre = vecs[0].astype(f32); lim = vecs[1].astype(f32)
        dt = jnp.exp(vecs[2].astype(f32)).astype(bf16).astype(f32)
        dsk = vecs[3].astype(f32)
        dsk_row = jnp.concatenate([dsk[j:j+1] for j in range(4)], axis=1)
        mag = jnp.exp(dt*lre); ang = dt*lim
        ar4 = mag*jnp.cos(ang); ai4 = mag*jnp.sin(ang)
        den = lre*lre + lim*lim
        nr = ar4 - 1.0
        gr4 = (nr*lre + ai4*lim)/den; gi4 = (ai4*lre - nr*lim)/den
        pr, pi = ar4, ai4
        for _ in range(logT):
            pr, pi = cmul(pr, pi, pr, pi)
        p2r, p2i = cmul(pr, pi, pr, pi)
        p4r, p4i = cmul(p2r, p2i, p2r, p2i)
        bc = lambda v, j: jnp.broadcast_to(v[j:j+1], (8, 128))
        sub = lax.broadcasted_iota(jnp.int32, (8, 128), 0)

        def ln_rows(b, r0, n, z=None):
            xb = b16(xv[b, pl.ds(r0//2, n//2), :]).astype(f32)
            if z is not None:
                xb = xb + jnp.concatenate([jnp.concatenate([z]*4, axis=1)]*(n//8), axis=0)
            if 'l' in ablate:
                xn = xb
            else:
                m = jnp.mean(xb, axis=-1, keepdims=True)
                xc = xb - m
                v = jnp.mean(xc*xc, axis=-1, keepdims=True)
                xn = xc * lax.rsqrt(v + 1e-5)
            xn_s[b, pl.ds(r0, n), :] = xn.astype(bf16)
            base_s[b, pl.ds(r0, n), :] = xb + xn*dsk_row
            return xn
        def ln(b, r0=0, n=R, z=None):
            return [ln_rows(b, r, lnch, z) for r in range(r0, r0+n, lnch)]

        def ustore(b, part, u, j0, r0):
            nr_, nc = u.shape
            for j in range(nc // 128):
                for s in range(8):
                    lo = max(s*T, r0); hi = min((s+1)*T, r0 + nr_)
                    if hi > lo:
                        us[b, part+j0+j, pl.ds(s*PU + lo - s*T, hi - lo), :] = u[lo-r0:hi-r0, j*128:(j+1)*128]
        def umat(b):
            xn = xn_s[b]
            for part, w in ((0, bre_v), (4, bim_v)):
                u = lax.dot_general(xn, b16(w[...]), NT, preferred_element_type=f32)
                ustore(b, part, u, 0, 0)
        def block0_head():
            M0 = R // m0
            done = [False]*nx0
            def need_rows(r1, z):
                for i in range(nx0):
                    if i*R0 < r1 and not done[i]:
                        cx0[i].wait(); ln(0, i*R0, R0, z); done[i] = True
            zrel = None
            for h in range(m0):
                need_rows((h+1)*M0, zrel)
                xn = xn_s[0, pl.ds(h*M0, M0), :]
                for i in range(nb):
                    if h == 0: cbre[i].wait()
                    u = lax.dot_general(xn, b16(bre_v[pl.ds(i*PB, PB), :]), NT, preferred_element_type=f32)
                    ustore(0, 0, u, i*(4//nb), h*M0)
                    if i == 0 and hdep: zrel = dep0(u[0:8, 0:128])
            cbim.wait()
            xn = xn_s[0]
            u = lax.dot_general(xn, b16(bim_v[...]), NT, preferred_element_type=f32)
            ustore(0, 4, u, 0, 0)

        def scan(b, carry, rel=None):
            if 's' in ablate:
                for j in range(8):
                    for s_ in range(8):
                        hs[b, j, pl.ds(s_*PH, T//2), :] = pltpu.bitcast(us[b, j, pl.ds(s_*PU, T//2), :], u32)
                return carry
            ar = [bc(ar4, j) for j in range(4)]; ai = [bc(ai4, j) for j in range(4)]
            er = [None]*4; ei = [None]*4
            seg1 = {}; seg2 = {}
            if rel is not None:
                for n_, k in enumerate(pace): seg1[(n_*T)//len(pace)] = k
                for n_, k in enumerate(pace2): seg2[(n_*(T//2))//len(pace2)] = k
            for t in range(T):
                if t in seg1:
                    z = rel(seg1[t])
                    if t == 0:
                        ar = [a_ + z for a_ in ar]
                    else:
                        er = [e_ + z for e_ in er]
                for j in range(4):
                    ur = us[b, j, pl.ds(t, 8, stride=PU), :]
                    ui = us[b, 4+j, pl.ds(t, 8, stride=PU), :]
                    if t == 0:
                        er[j], ei[j] = ur, ui
                    else:
                        er[j], ei[j] = ar[j]*er[j] - ai[j]*ei[j] + ur, ar[j]*ei[j] + ai[j]*er[j] + ui
            hr = [None]*4; hi = [None]*4
            newc = []
            for j in range(4):
                if carry is None:
                    zr = jnp.where(sub == 0, 0.0, pltpu.roll(er[j], 1, 0))
                    zi = jnp.where(sub == 0, 0.0, pltpu.roll(ei[j], 1, 0))
                else:
                    zr = pltpu.roll(jnp.where(sub == 7, carry[j][0], er[j]), 1, 0)
                    zi = pltpu.roll(jnp.where(sub == 7, carry[j][1], ei[j]), 1, 0)
                for k, (qr, qi) in ((1, (pr, pi)), (2, (p2r, p2i)), (4, (p4r, p4i))):
                    mr = jnp.where(sub >= k, bc(qr, j), 0.0); mi = jnp.where(sub >= k, bc(qi, j), 0.0)
                    sr = pltpu.roll(zr, k, 0); si = pltpu.roll(zi, k, 0)
                    zr, zi = zr + (mr*sr - mi*si), zi + (mr*si + mi*sr)
                hr[j], hi[j] = zr, zi
                tr, ti = cmul(bc(pr, j), bc(pi, j), zr, zi)
                newc.append((er[j] + tr, ei[j] + ti))
            for tau in range(T//2):
                if tau in seg2:
                    z = rel(seg2[tau])
                    hr = [h_ + z for h_ in hr]
                for j in range(4):
                    outs = []
                    for bb in range(2):
                        t = 2*tau + bb
                        ur = us[b, j, pl.ds(t, 8, stride=PU), :]
                        ui = us[b, 4+j, pl.ds(t, 8, stride=PU), :]
                        hr[j], hi[j] = ar[j]*hr[j] - ai[j]*hi[j] + ur, ar[j]*hi[j] + ai[j]*hr[j] + ui
                        outs.append((hr[j], hi[j]))
                    hs[b, j, pl.ds(tau, 8, stride=PH), :] = pltpu.pack_elementwise([outs[0][0], outs[1][0]], packed_dtype=bf16)
                    hs[b, 4+j, pl.ds(tau, 8, stride=PH), :] = pltpu.pack_elementwise([outs[0][1], outs[1][1]], packed_dtype=bf16)
            return newc

        def cprep():
            CH = cch
            for j in range(4):
                sl = slice(j*128, (j+1)*128)
                g_r = 2.0*gr4[j:j+1]; g_i = 2.0*gi4[j:j+1]
                ng_r = -g_r; ng_i = -g_i
                for r in range(0, D//2, CH//2):
                    cr = b16(cre_v[pl.ds(r, CH//2), sl]).astype(f32); ci = b16(cim_v[pl.ds(r, CH//2), sl]).astype(f32)
                    cp_v[pl.ds(r, CH//2), sl] = w32((cr*g_r - ci*g_i).astype(bf16))
                    cp_v[pl.ds(r, CH//2), pl.ds(512 + j*128, 128)] = w32((cr*ng_i + ci*ng_r).astype(bf16))

        def ffn1(b, mid=None):
            xn = xn_s[b]
            with sc("gate", b):
                if b == 0:
                    gs = []
                    for i in range(len(gch)):
                        cwg[i].wait()
                        gs.append(lax.dot_general(xn, b16(wg_v[pl.ds(goff[i]//2, gch[i]//2), :]), NT, preferred_element_type=f32))
                    g = jnp.concatenate(gs, axis=1) if len(gs) > 1 else gs[0]
                    cwu.wait()
                else:
                    g = lax.dot_general(xn, b16(wg_v[...]), NT, preferred_element_type=f32)
            if mid is not None: mid(g)
            with sc("up", b):
                u = lax.dot_general(xn, b16(wu_v[...]), NT, preferred_element_type=f32)
                a_s[b] = ((g*u) if 'g' in ablate else gelu_mul(g, u)).astype(bf16)

        def final(b, xns=None):
            with sc("down", b):
                acc = base_s[b] + lax.dot_general(a_s[b], b16(wd_v[...]), NN, preferred_element_type=f32)
                if xns is not None:
                    q = len(xns)//4
                    cols = []
                    for j in range(4):
                        z = dep0(xns[j*q][0:8, 0:128])
                        for i in range(1, q): z = z + dep0(xns[j*q+i][0:8, 0:128])
                        cj = acc[:, j*128:(j+1)*128]
                        cols.append(jnp.concatenate([cj[:R-8], cj[R-8:] + z], axis=0))
                    acc = jnp.concatenate(cols, axis=1)
            cs = []
            with sc("C", b):
                H = jnp.concatenate([
                        jnp.concatenate([pltpu.bitcast(hs[b, jj, pl.ds(s*PH, T//2), :], bf16) for s in range(8)], axis=0)
                        for jj in range(8)], axis=1)
                n = nsplit if b == nrun-1 else 1
                Wn = D // n
                for i in range(n):
                    a2 = acc[:, i*Wn:(i+1)*Wn] + lax.dot_general(H, b16(cp_v[pl.ds(i*Wn//2, Wn//2), :]), NT, preferred_element_type=f32)
                    ov[b, :, pl.ds(i*Wn, Wn)] = a2.astype(bf16)
                    c = pltpu.make_async_copy(ov.at[b, :, pl.ds(i*Wn, Wn)], out_hbm.at[pl.ds(b*R, R), pl.ds(i*Wn, Wn)], osem)
                    c.start(); cs.append(c)
            return cs

        outs = []
        carry = None
        for b in range(nrun):
            with sc("U", b):
                if b == 0: block0_head()
                else: umat(b)
            if pace:
                cbox = [carry]
                def mid(g):
                    rel = lambda k: dep0(g[prow:prow+8, k*128:min((k+1)*128, F)] if (k+1)*128 <= F else g[prow:prow+8, F-128:F])
                    cbox[0] = scan(b, cbox[0], rel)
                ffn1(b, mid)
                carry = cbox[0]
            else:
                carry = scan(b, carry)
                ffn1(b)
            if b == 0:
                cwd.wait()
                cc.wait(); cprep()
            if b + 1 < NB: cx[b+1].wait()
            xns = ln(b+1) if b + 1 < nrun else None
            outs += final(b, xns if lnd else None)
        if cur[0] is not None: cur[0].__exit__(None, None, None); cur[0] = None
        with scope("tail"):
            for c in outs: c.wait()

    def f(A_x, A_Lambda_re, A_Lambda_im, A_B_re, A_B_im, A_C_re, A_C_im, A_log_dt, A_Dskip, B_x, B_w_gate, B_w_up, B_w_down):
        hbm = pl.BlockSpec(memory_space=pltpu.HBM)
        out = pl.pallas_call(kernel,
            out_shape=jax.ShapeDtypeStruct((L, D), bf16),
            in_specs=[hbm]*12, out_specs=hbm,
            scratch_shapes=[
                pltpu.VMEM((NB, R//2, D), u32),
                pltpu.VMEM((4, 4, 128), bf16),
                pltpu.VMEM((P//2, D), u32), pltpu.VMEM((P//2, D), u32),
                pltpu.VMEM((D//2, P), u32), pltpu.VMEM((D//2, P), u32),
                pltpu.VMEM((D//2, 2*P), u32),
                pltpu.VMEM((F//2, D), u32), pltpu.VMEM((F//2, D), u32), pltpu.VMEM((F//2, D), u32),
                pltpu.VMEM((NB, R, D), bf16),
                pltpu.VMEM((NB, R, D), f32),
                pltpu.VMEM((NB, 8, 8*PU, 128), f32),
                pltpu.VMEM((NB, 8, 8*PH, 128), u32),
                pltpu.VMEM((NB, R, F), bf16),
                pltpu.VMEM((NB, R, D), bf16),
                pltpu.SemaphoreType.DMA((NSEM,)),
            ],
            compiler_params=pltpu.CompilerParams(vmem_limit_bytes=vmem_limit, flags=flags, disable_semaphore_checks=dsc),
            name="ssm_ffn",
        )(A_x.reshape(L, D), A_Lambda_re.reshape(4,128), A_Lambda_im.reshape(4,128), A_log_dt.reshape(4,128), A_Dskip.reshape(4,128),
          A_B_re, A_B_im, A_C_re, A_C_im, B_w_gate.T, B_w_up.T, B_w_down)
        return out.reshape(1, L, D)
    return f


_impl = make(nx0=4, m0=4, nb=2, order='x0 v b0 b1 x1 x2 x3', pace=(), flags={'XLA_TPU_RESCHEDULE_DMA_DONES': True})


@jax.jit
def pallas_parallel_sum__ssm_conv_s5__geglu_ffn__prompt_kernel(
    A_x, A_Lambda_re, A_Lambda_im, A_B_re, A_B_im, A_C_re, A_C_im, A_log_dt, A_Dskip,
    B_x, B_w_gate, B_w_up, B_w_down,
):
    return _impl(A_x, A_Lambda_re, A_Lambda_im, A_B_re, A_B_im, A_C_re, A_C_im, A_log_dt, A_Dskip,
                 B_x, B_w_gate, B_w_up, B_w_down)
```

```python
import numpy as np
import jax
import jax.numpy as jnp
from jax import lax
from jax.experimental import pallas as pl
from jax.experimental.pallas import tpu as pltpu

L, D, P, F = 2048, 512, 512, 1376
R = 512
NB = L // R
T = R // 8
PU = T + 1
SKEW_ROWS = -(-9 * PU // 8) * 8
NX0 = 4
GCH = (256, 256, 384, 480)
NBI = 2
LNCH = 32
HEAD_JOBS = ((0, 0), (1, 0), (0, 1), (1, 1), (2, 0), (2, 1), (0, 2), (1, 2),
             (2, 2), (3, 0), (3, 1), (3, 2), (0, 3), (1, 3), (2, 3), (3, 3))
NSEM = 1 + 2 * NX0 + NBI + len(GCH) + 3 + (NB - 1) + 1

NT = (((1,), (1,)), ((), ()))
NN = (((1,), (0,)), ((), ()))
C0 = float(np.sqrt(2 / np.pi))
C1 = float(np.sqrt(2 / np.pi) * 0.044715)
f32, bf16, u32 = jnp.float32, jnp.bfloat16, jnp.uint32


def _b16(w):
    return pltpu.bitcast(w, bf16)


def _w32(v):
    return pltpu.bitcast(v, u32)


def _dot(a, b, dims):
    return lax.dot_general(a, b, dims, preferred_element_type=f32)


def _geglu(g, u):
    inner = g * (C0 + C1 * (g * g))
    return (0.5 * g * u) * (1.0 + jnp.tanh(inner))


def _cmul(ar, ai, br, bi):
    return ar * br - ai * bi, ar * bi + ai * br


def _dep0(v):
    z = jnp.minimum(pltpu.bitcast(v, jnp.int32) & 1, 0)
    return pltpu.bitcast(z, f32)


def _kernel(x_hbm, lre_hbm, lim_hbm, ldt_hbm, dsk_hbm, bre_hbm, bim_hbm, cre_hbm, cim_hbm,
            wg_hbm, wu_hbm, wd_hbm, out_hbm,
            xv, vecs, bre_v, bim_v, cre_v, cim_v, cp_v, wg_v, wu_v, wd_v,
            xn_s, base_s, us, hp, ys, a_s, ov, sems):
    nsem = [0]

    def start(pairs):
        sem = sems.at[nsem[0]]
        nsem[0] += 1
        cps = [pltpu.make_async_copy(s, d, sem) for s, d in pairs]
        for c in cps:
            c.start()
        return cps

    def wait(cps):
        for c in cps:
            c.wait()

    x_hbm, bre_hbm, bim_hbm, cre_hbm, cim_hbm, wg_hbm, wu_hbm, wd_hbm = [
        r.bitcast(u32) for r in (x_hbm, bre_hbm, bim_hbm, cre_hbm, cim_hbm, wg_hbm, wu_hbm, wd_hbm)]
    M0 = R // NX0
    PB = P // NX0 // 2
    PBI = P // NBI // 2
    cx0, cbre, cv = [], [], None
    for i in range(NX0):
        cx0.append(start([(x_hbm.at[pl.ds(i * M0 // 2, M0 // 2)], xv.at[0, pl.ds(i * M0 // 2, M0 // 2)])]))
        if i == 0:
            cv = start([(r, vecs.at[k]) for k, r in enumerate((lre_hbm, lim_hbm, ldt_hbm, dsk_hbm))])
        cbre.append(start([(bre_hbm.at[pl.ds(i * PB, PB)], bre_v.at[pl.ds(i * PB, PB)])]))
    cbim = [start([(bim_hbm.at[pl.ds(i * PBI, PBI)], bim_v.at[pl.ds(i * PBI, PBI)])]) for i in range(NBI)]
    goff = [sum(GCH[:i]) for i in range(len(GCH))]
    cwg = [start([(wg_hbm.at[pl.ds(o // 2, n // 2)], wg_v.at[pl.ds(o // 2, n // 2)])])
           for o, n in zip(goff, GCH)]
    cwu = start([(wu_hbm, wu_v)])
    cwd = start([(wd_hbm, wd_v)])
    cc = start([(cre_hbm, cre_v), (cim_hbm, cim_v)])
    cx = [None] + [start([(x_hbm.at[pl.ds(b * R // 2, R // 2)], xv.at[b])]) for b in range(1, NB)]
    osem = sems.at[nsem[0]]

    wait(cv)
    lre = vecs[0].astype(f32)
    lim = vecs[1].astype(f32)
    dt = jnp.exp(vecs[2].astype(f32)).astype(bf16).astype(f32)
    dsk = vecs[3].astype(f32)
    dsk_row = jnp.concatenate([dsk[j:j + 1] for j in range(4)], axis=1)
    mag = jnp.exp(dt * lre)
    ang = dt * lim
    ar4 = mag * jnp.cos(ang)
    ai4 = mag * jnp.sin(ang)
    den = lre * lre + lim * lim
    nr = ar4 - 1.0
    gr4 = (nr * lre + ai4 * lim) / den
    gi4 = (ai4 * lre - nr * lim) / den
    p1 = (ar4, ai4)
    for _ in range(T.bit_length() - 1):
        p1 = _cmul(*p1, *p1)
    p2 = _cmul(*p1, *p1)
    p4 = _cmul(*p2, *p2)
    sub = lax.broadcasted_iota(jnp.int32, (8, 128), 0)

    def bc(v, j):
        return jnp.broadcast_to(v[j:j + 1], (8, 128))

    def layernorm(b, r0, n):
        outs = []
        for r in range(r0, r0 + n, LNCH):
            xb = _b16(xv[b, pl.ds(r // 2, LNCH // 2), :]).astype(f32)
            m = jnp.mean(xb, axis=-1, keepdims=True)
            xc = xb - m
            v = jnp.mean(xc * xc, axis=-1, keepdims=True)
            xn = xc * lax.rsqrt(v + 1e-5)
            xn_s[b, pl.ds(r, LNCH), :] = xn.astype(bf16)
            base_s[b, pl.ds(r, LNCH), :] = xb + xn * dsk_row
            outs.append(xn)
        return outs

    def store_u(b, part, u, j0, r0):
        rows, cols = u.shape
        for j in range(cols // 128):
            for s in range(8):
                lo, hi = max(s * T, r0), min((s + 1) * T, r0 + rows)
                if hi > lo:
                    us[b, part + j0 + j, pl.ds(s * PU + lo - s * T, hi - lo), :] = (
                        u[lo - r0:hi - r0, j * 128:(j + 1) * 128])

    def bu(b):
        if b == 0:
            x_done, b_done = [False] * NX0, [False] * NX0
            for h, i in HEAD_JOBS:
                for k in range(h + 1):
                    if not x_done[k]:
                        wait(cx0[k])
                        layernorm(0, k * M0, M0)
                        x_done[k] = True
                if not b_done[i]:
                    wait(cbre[i])
                    b_done[i] = True
                u = _dot(xn_s[0, pl.ds(h * M0, M0), :], _b16(bre_v[pl.ds(i * PB, PB), :]), NT)
                store_u(0, 0, u, i * (4 // NX0), h * M0)
            xn = xn_s[0]
            for i in range(NBI):
                wait(cbim[i])
                store_u(0, 4, _dot(xn, _b16(bim_v[pl.ds(i * PBI, PBI), :]), NT), i * (4 // NBI), 0)
        else:
            xn = xn_s[b]
            store_u(b, 0, _dot(xn, _b16(bre_v[...]), NT), 0, 0)
            store_u(b, 4, _dot(xn, _b16(bim_v[...]), NT), 0, 0)

    def scan(b, carry):
        ar = [bc(ar4, j) for j in range(4)]
        ai = [bc(ai4, j) for j in range(4)]

        def step(t, j, hr, hi):
            ur = us[b, j, pl.ds(t, 8, stride=PU), :]
            ui = us[b, 4 + j, pl.ds(t, 8, stride=PU), :]
            if hr is None:
                return ur, ui
            return ar[j] * hr - ai[j] * hi + ur, ar[j] * hi + ai[j] * hr + ui

        er, ei = [None] * 4, [None] * 4
        for t in range(T):
            for j in range(4):
                er[j], ei[j] = step(t, j, er[j], ei[j])
        hr, hi, new_carry = [None] * 4, [None] * 4, []
        for j in range(4):
            if carry is None:
                zr = jnp.where(sub == 0, 0.0, pltpu.roll(er[j], 1, 0))
                zi = jnp.where(sub == 0, 0.0, pltpu.roll(ei[j], 1, 0))
            else:
                zr = pltpu.roll(jnp.where(sub == 7, carry[j][0], er[j]), 1, 0)
                zi = pltpu.roll(jnp.where(sub == 7, carry[j][1], ei[j]), 1, 0)
            for k, (qr, qi) in ((1, p1), (2, p2), (4, p4)):
                mr = jnp.where(sub >= k, bc(qr, j), 0.0)
                mi = jnp.where(sub >= k, bc(qi, j), 0.0)
                sr = pltpu.roll(zr, k, 0)
                si = pltpu.roll(zi, k, 0)
                zr, zi = zr + (mr * sr - mi * si), zi + (mr * si + mi * sr)
            hr[j], hi[j] = zr, zi
            tr, ti = _cmul(bc(p1[0], j), bc(p1[1], j), zr, zi)
            new_carry.append((er[j] + tr, ei[j] + ti))
        for tau in range(T // 2):
            rows = []
            for t in (2 * tau, 2 * tau + 1):
                for j in range(4):
                    hr[j], hi[j] = step(t, j, hr[j], hi[j])
                rows.append(jnp.concatenate(hr + hi, axis=1))
            hp[b, pl.ds(16 * tau, 16), :] = jnp.concatenate(rows, axis=0).astype(bf16)
        return new_carry

    def prep_c():
        CH = 32
        for j in range(4):
            sl = pl.ds(j * 128, 128)
            g_r = 2.0 * gr4[j:j + 1]
            g_i = 2.0 * gi4[j:j + 1]
            ng_r, ng_i = -g_r, -g_i
            for r in range(0, D // 2, CH // 2):
                cr = _b16(cre_v[pl.ds(r, CH // 2), sl]).astype(f32)
                ci = _b16(cim_v[pl.ds(r, CH // 2), sl]).astype(f32)
                cp_v[pl.ds(r, CH // 2), sl] = _w32((cr * g_r - ci * g_i).astype(bf16))
                cp_v[pl.ds(r, CH // 2), pl.ds(P + j * 128, 128)] = _w32((cr * ng_i + ci * ng_r).astype(bf16))

    def gate_up(b):
        xn = xn_s[b]
        if b == 0:
            gs = []
            for i, (o, n) in enumerate(zip(goff, GCH)):
                wait(cwg[i])
                gs.append(_dot(xn, _b16(wg_v[pl.ds(o // 2, n // 2), :]), NT))
            g = jnp.concatenate(gs, axis=1)
            wait(cwu)
        else:
            g = _dot(xn, _b16(wg_v[...]), NT)
        u = _dot(xn, _b16(wu_v[...]), NT)
        a_s[b] = _geglu(g, u).astype(bf16)

    def finish(b, xn_next):
        acc = base_s[b] + _dot(a_s[b], _b16(wd_v[...]), NN)
        if xn_next is not None:
            q = len(xn_next) // 4
            cols = []
            for j in range(4):
                z = _dep0(xn_next[j * q][0:8, 0:128])
                for i in range(1, q):
                    z = z + _dep0(xn_next[j * q + i][0:8, 0:128])
                cj = acc[:, j * 128:(j + 1) * 128]
                cols.append(jnp.concatenate([cj[:R - 8], cj[R - 8:] + z], axis=0))
            acc = jnp.concatenate(cols, axis=1)
        h = hp[b]
        last = b == NB - 1
        n = 4 if last else 1
        Wn = D // n
        cps = []
        for i in range(n):
            y = _dot(h, _b16(cp_v[pl.ds(i * Wn // 2, Wn // 2), :]), NT)
            cols = []
            for jj in range(Wn // 128):
                jg = i * (Wn // 128) + jj
                for t in range(T):
                    ys[b, jg, pl.ds(t, 8, stride=PU), :] = y[8 * t:8 * t + 8, jj * 128:(jj + 1) * 128]
                cols.append(jnp.concatenate([ys[b, jg, pl.ds(s * PU, T), :] for s in range(8)], axis=0))
            y = jnp.concatenate(cols, axis=1) if len(cols) > 1 else cols[0]
            o = acc[:, i * Wn:(i + 1) * Wn] + y
            nq = 4 if (last and i == n - 1) else 1
            Rq = R // nq
            for qi in range(nq):
                ov[b, pl.ds(qi * Rq, Rq), pl.ds(i * Wn, Wn)] = o[qi * Rq:(qi + 1) * Rq].astype(bf16)
                c = pltpu.make_async_copy(ov.at[b, pl.ds(qi * Rq, Rq), pl.ds(i * Wn, Wn)],
                                          out_hbm.at[pl.ds(b * R + qi * Rq, Rq), pl.ds(i * Wn, Wn)], osem)
                c.start()
                cps.append(c)
        return cps

    outs, carry = [], None
    for b in range(NB):
        bu(b)
        carry = scan(b, carry)
        gate_up(b)
        if b == 0:
            wait(cwd)
            wait(cc)
            prep_c()
        xn_next = None
        if b + 1 < NB:
            wait(cx[b + 1])
            xn_next = layernorm(b + 1, 0, R)
        outs += finish(b, xn_next)
    wait(outs)


@jax.jit
def pallas_parallel_sum__ssm_conv_s5__geglu_ffn__prompt_kernel(
    A_x: jax.Array,
    A_Lambda_re: jax.Array,
    A_Lambda_im: jax.Array,
    A_B_re: jax.Array,
    A_B_im: jax.Array,
    A_C_re: jax.Array,
    A_C_im: jax.Array,
    A_log_dt: jax.Array,
    A_Dskip: jax.Array,
    B_x: jax.Array,
    B_w_gate: jax.Array,
    B_w_up: jax.Array,
    B_w_down: jax.Array,
):
    del B_x
    hbm = pl.BlockSpec(memory_space=pltpu.HBM)
    out = pl.pallas_call(
        _kernel,
        out_shape=jax.ShapeDtypeStruct((L, D), bf16),
        in_specs=[hbm] * 12,
        out_specs=hbm,
        scratch_shapes=[
            pltpu.VMEM((NB, R // 2, D), u32),
            pltpu.VMEM((4, 4, 128), bf16),
            pltpu.VMEM((P // 2, D), u32),
            pltpu.VMEM((P // 2, D), u32),
            pltpu.VMEM((D // 2, P), u32),
            pltpu.VMEM((D // 2, P), u32),
            pltpu.VMEM((D // 2, 2 * P), u32),
            pltpu.VMEM((F // 2, D), u32),
            pltpu.VMEM((F // 2, D), u32),
            pltpu.VMEM((F // 2, D), u32),
            pltpu.VMEM((NB, R, D), bf16),
            pltpu.VMEM((NB, R, D), f32),
            pltpu.VMEM((NB, 8, SKEW_ROWS, 128), f32),
            pltpu.VMEM((NB, R, 2 * P), bf16),
            pltpu.VMEM((NB, 4, SKEW_ROWS, 128), f32),
            pltpu.VMEM((NB, R, F), bf16),
            pltpu.VMEM((NB, R, D), bf16),
            pltpu.SemaphoreType.DMA((NSEM,)),
        ],
        compiler_params=pltpu.CompilerParams(
            vmem_limit_bytes=100 * 2**20,
            disable_semaphore_checks=True,
            flags={"XLA_TPU_RESCHEDULE_DMA_DONES": True},
        ),
        name="ssm_geglu",
    )(A_x.reshape(L, D),
      A_Lambda_re.reshape(4, 128), A_Lambda_im.reshape(4, 128),
      A_log_dt.reshape(4, 128), A_Dskip.reshape(4, 128),
      A_B_re, A_B_im, A_C_re, A_C_im, B_w_gate.T, B_w_up.T, B_w_down)
    return out.reshape(1, L, D)
```

```python
import numpy as np
import jax
import jax.numpy as jnp
from jax import lax
from jax.experimental import pallas as pl
from jax.experimental.pallas import tpu as pltpu

L, D, P, F = 2048, 512, 512, 1376
R = 512
NB = L // R
T = R // 8
PU = T + 1
SKEW_ROWS = -(-9 * PU // 8) * 8
NX0 = 4
GCH = (256, 256, 384, 480)
UCH = (256, 256, 864)
NBI = 2
LNCH = 32
HEAD_JOBS = ((0, 0), (1, 0), (0, 1), (1, 1), (2, 0), (2, 1), (0, 2), (1, 2),
             (2, 2), (3, 0), (3, 1), (3, 2), (0, 3), (1, 3), (2, 3), (3, 3))
NSEM = 1 + 2 * NX0 + NBI + len(GCH) + len(UCH) + 2 + (NB - 1) + 1

NT = (((1,), (1,)), ((), ()))
NN = (((1,), (0,)), ((), ()))
C0 = float(np.sqrt(2 / np.pi))
C1 = float(np.sqrt(2 / np.pi) * 0.044715)
f32, bf16, u32 = jnp.float32, jnp.bfloat16, jnp.uint32


def _b16(w):
    return pltpu.bitcast(w, bf16)


def _w32(v):
    return pltpu.bitcast(v, u32)


def _dot(a, b, dims):
    return lax.dot_general(a, b, dims, preferred_element_type=f32)


def _geglu(g, u):
    inner = g * (C0 + C1 * (g * g))
    return (0.5 * g * u) * (1.0 + jnp.tanh(inner))


def _cmul(ar, ai, br, bi):
    return ar * br - ai * bi, ar * bi + ai * br


def _dep0(v):
    z = jnp.minimum(pltpu.bitcast(v, jnp.int32) & 1, 0)
    return pltpu.bitcast(z, f32)


def _kernel(x_hbm, lre_hbm, lim_hbm, ldt_hbm, dsk_hbm, bre_hbm, bim_hbm, cre_hbm, cim_hbm,
            wg_hbm, wu_hbm, wd_hbm, out_hbm,
            xv, vecs, bre_v, bim_v, cre_v, cim_v, cp_v, wg_v, wu_v, wd_v,
            xn_s, base_s, us, hp, ys, a_s, ov, sems):
    nsem = [0]

    def start(pairs):
        sem = sems.at[nsem[0]]
        nsem[0] += 1
        cps = [pltpu.make_async_copy(s, d, sem) for s, d in pairs]
        for c in cps:
            c.start()
        return cps

    def wait(cps):
        for c in cps:
            c.wait()

    x_hbm, bre_hbm, bim_hbm, cre_hbm, cim_hbm, wg_hbm, wu_hbm, wd_hbm = [
        r.bitcast(u32) for r in (x_hbm, bre_hbm, bim_hbm, cre_hbm, cim_hbm, wg_hbm, wu_hbm, wd_hbm)]
    M0 = R // NX0
    PB = P // NX0 // 2
    PBI = P // NBI // 2
    cx0, cbre, cv = [], [], None
    for i in range(NX0):
        cx0.append(start([(x_hbm.at[pl.ds(i * M0 // 2, M0 // 2)], xv.at[0, pl.ds(i * M0 // 2, M0 // 2)])]))
        if i == 0:
            cv = start([(r, vecs.at[k]) for k, r in enumerate((lre_hbm, lim_hbm, ldt_hbm, dsk_hbm))])
        cbre.append(start([(bre_hbm.at[pl.ds(i * PB, PB)], bre_v.at[pl.ds(i * PB, PB)])]))
    cbim = [start([(bim_hbm.at[pl.ds(i * PBI, PBI)], bim_v.at[pl.ds(i * PBI, PBI)])]) for i in range(NBI)]
    goff = [sum(GCH[:i]) for i in range(len(GCH))]
    cwg = [start([(wg_hbm.at[pl.ds(o // 2, n // 2)], wg_v.at[pl.ds(o // 2, n // 2)])])
           for o, n in zip(goff, GCH)]
    cc = start([(cre_hbm, cre_v), (cim_hbm, cim_v)])
    uoff = [sum(UCH[:i]) for i in range(len(UCH))]
    cwu = [start([(wu_hbm.at[pl.ds(o // 2, n // 2)], wu_v.at[pl.ds(o // 2, n // 2)])])
           for o, n in zip(uoff, UCH)]
    cwd = start([(wd_hbm, wd_v)])
    cx = [None] + [start([(x_hbm.at[pl.ds(b * R // 2, R // 2)], xv.at[b])]) for b in range(1, NB)]
    osem = sems.at[nsem[0]]

    wait(cv)
    lre = vecs[0].astype(f32)
    lim = vecs[1].astype(f32)
    dt = jnp.exp(vecs[2].astype(f32)).astype(bf16).astype(f32)
    dsk = vecs[3].astype(f32)
    dsk_row = jnp.concatenate([dsk[j:j + 1] for j in range(4)], axis=1)
    mag = jnp.exp(dt * lre)
    ang = dt * lim
    ar4 = mag * jnp.cos(ang)
    ai4 = mag * jnp.sin(ang)
    den = lre * lre + lim * lim
    nr = ar4 - 1.0
    gr4 = (nr * lre + ai4 * lim) / den
    gi4 = (ai4 * lre - nr * lim) / den
    p1 = (ar4, ai4)
    for _ in range(T.bit_length() - 1):
        p1 = _cmul(*p1, *p1)
    p2 = _cmul(*p1, *p1)
    p4 = _cmul(*p2, *p2)
    sub = lax.broadcasted_iota(jnp.int32, (8, 128), 0)

    def bc(v, j):
        return jnp.broadcast_to(v[j:j + 1], (8, 128))

    def layernorm(b, r0, n):
        outs = []
        for r in range(r0, r0 + n, LNCH):
            xb = _b16(xv[b, pl.ds(r // 2, LNCH // 2), :]).astype(f32)
            m = jnp.mean(xb, axis=-1, keepdims=True)
            xc = xb - m
            v = jnp.mean(xc * xc, axis=-1, keepdims=True)
            xn = xc * lax.rsqrt(v + 1e-5)
            xn_s[b, pl.ds(r, LNCH), :] = xn.astype(bf16)
            base_s[b, pl.ds(r, LNCH), :] = xb + xn * dsk_row
            outs.append(xn)
        return outs

    def store_u(b, part, u, j0, r0):
        rows, cols = u.shape
        for j in range(cols // 128):
            for s in range(8):
                lo, hi = max(s * T, r0), min((s + 1) * T, r0 + rows)
                if hi > lo:
                    us[b, part + j0 + j, pl.ds(s * PU + lo - s * T, hi - lo), :] = (
                        u[lo - r0:hi - r0, j * 128:(j + 1) * 128])

    def bu(b):
        if b == 0:
            x_done, b_done = [False] * NX0, [False] * NX0
            for h, i in HEAD_JOBS:
                for k in range(h + 1):
                    if not x_done[k]:
                        wait(cx0[k])
                        layernorm(0, k * M0, M0)
                        x_done[k] = True
                if not b_done[i]:
                    wait(cbre[i])
                    b_done[i] = True
                u = _dot(xn_s[0, pl.ds(h * M0, M0), :], _b16(bre_v[pl.ds(i * PB, PB), :]), NT)
                store_u(0, 0, u, i * (4 // NX0), h * M0)
            xn = xn_s[0]
            for i in range(NBI):
                wait(cbim[i])
                store_u(0, 4, _dot(xn, _b16(bim_v[pl.ds(i * PBI, PBI), :]), NT), i * (4 // NBI), 0)
        else:
            xn = xn_s[b]
            store_u(b, 0, _dot(xn, _b16(bre_v[...]), NT), 0, 0)
            store_u(b, 4, _dot(xn, _b16(bim_v[...]), NT), 0, 0)

    def scan(b, carry):
        ar = [bc(ar4, j) for j in range(4)]
        ai = [bc(ai4, j) for j in range(4)]

        def step(t, j, hr, hi):
            ur = us[b, j, pl.ds(t, 8, stride=PU), :]
            ui = us[b, 4 + j, pl.ds(t, 8, stride=PU), :]
            if hr is None:
                return ur, ui
            return ar[j] * hr - ai[j] * hi + ur, ar[j] * hi + ai[j] * hr + ui

        er, ei = [None] * 4, [None] * 4
        for t in range(T):
            for j in range(4):
                er[j], ei[j] = step(t, j, er[j], ei[j])
        hr, hi, new_carry = [None] * 4, [None] * 4, []
        for j in range(4):
            if carry is None:
                zr = jnp.where(sub == 0, 0.0, pltpu.roll(er[j], 1, 0))
                zi = jnp.where(sub == 0, 0.0, pltpu.roll(ei[j], 1, 0))
            else:
                zr = pltpu.roll(jnp.where(sub == 7, carry[j][0], er[j]), 1, 0)
                zi = pltpu.roll(jnp.where(sub == 7, carry[j][1], ei[j]), 1, 0)
            for k, (qr, qi) in ((1, p1), (2, p2), (4, p4)):
                mr = jnp.where(sub >= k, bc(qr, j), 0.0)
                mi = jnp.where(sub >= k, bc(qi, j), 0.0)
                sr = pltpu.roll(zr, k, 0)
                si = pltpu.roll(zi, k, 0)
                zr, zi = zr + (mr * sr - mi * si), zi + (mr * si + mi * sr)
            hr[j], hi[j] = zr, zi
            tr, ti = _cmul(bc(p1[0], j), bc(p1[1], j), zr, zi)
            new_carry.append((er[j] + tr, ei[j] + ti))
        for tau in range(T // 2):
            rows = []
            for t in (2 * tau, 2 * tau + 1):
                for j in range(4):
                    hr[j], hi[j] = step(t, j, hr[j], hi[j])
                rows.append(jnp.concatenate(hr + hi, axis=1))
            hp[b, pl.ds(16 * tau, 16), :] = jnp.concatenate(rows, axis=0).astype(bf16)
        return new_carry

    def prep_c():
        CH = 32
        for j in range(4):
            sl = pl.ds(j * 128, 128)
            g_r = 2.0 * gr4[j:j + 1]
            g_i = 2.0 * gi4[j:j + 1]
            ng_r, ng_i = -g_r, -g_i
            for r in range(0, D // 2, CH // 2):
                cr = _b16(cre_v[pl.ds(r, CH // 2), sl]).astype(f32)
                ci = _b16(cim_v[pl.ds(r, CH // 2), sl]).astype(f32)
                cp_v[pl.ds(r, CH // 2), sl] = _w32((cr * g_r - ci * g_i).astype(bf16))
                cp_v[pl.ds(r, CH // 2), pl.ds(P + j * 128, 128)] = _w32((cr * ng_i + ci * ng_r).astype(bf16))

    def gate_up(b):
        xn = xn_s[b]

        def pieces(w_v, cps, offs, sizes):
            ys_ = []
            for c, o, n in zip(cps, offs, sizes):
                wait(c)
                ys_.append(_dot(xn, _b16(w_v[pl.ds(o // 2, n // 2), :]), NT))
            return jnp.concatenate(ys_, axis=1)

        if b == 0:
            g = pieces(wg_v, cwg, goff, GCH)
            wait(cc)
            prep_c()
            u = pieces(wu_v, cwu, uoff, UCH)
        else:
            g = _dot(xn, _b16(wg_v[...]), NT)
            u = _dot(xn, _b16(wu_v[...]), NT)
        a_s[b] = _geglu(g, u).astype(bf16)

    def finish(b, xn_next):
        acc = base_s[b] + _dot(a_s[b], _b16(wd_v[...]), NN)
        if xn_next is not None:
            q = len(xn_next) // 4
            cols = []
            for j in range(4):
                z = _dep0(xn_next[j * q][0:8, 0:128])
                for i in range(1, q):
                    z = z + _dep0(xn_next[j * q + i][0:8, 0:128])
                cj = acc[:, j * 128:(j + 1) * 128]
                cols.append(jnp.concatenate([cj[:R - 8], cj[R - 8:] + z], axis=0))
            acc = jnp.concatenate(cols, axis=1)
        h = hp[b]
        last = b == NB - 1
        n = 4 if last else 1
        Wn = D // n
        cps = []
        for i in range(n):
            y = _dot(h, _b16(cp_v[pl.ds(i * Wn // 2, Wn // 2), :]), NT)
            cols = []
            for jj in range(Wn // 128):
                jg = i * (Wn // 128) + jj
                for t in range(T):
                    ys[b, jg, pl.ds(t, 8, stride=PU), :] = y[8 * t:8 * t + 8, jj * 128:(jj + 1) * 128]
                cols.append(jnp.concatenate([ys[b, jg, pl.ds(s * PU, T), :] for s in range(8)], axis=0))
            y = jnp.concatenate(cols, axis=1) if len(cols) > 1 else cols[0]
            o = acc[:, i * Wn:(i + 1) * Wn] + y
            nq = 4 if (last and i == n - 1) else 1
            Rq = R // nq
            for qi in range(nq):
                ov[b, pl.ds(qi * Rq, Rq), pl.ds(i * Wn, Wn)] = o[qi * Rq:(qi + 1) * Rq].astype(bf16)
                c = pltpu.make_async_copy(ov.at[b, pl.ds(qi * Rq, Rq), pl.ds(i * Wn, Wn)],
                                          out_hbm.at[pl.ds(b * R + qi * Rq, Rq), pl.ds(i * Wn, Wn)], osem)
                c.start()
                cps.append(c)
        return cps

    outs, carry = [], None
    for b in range(NB):
        bu(b)
        carry = scan(b, carry)
        gate_up(b)
        if b == 0:
            wait(cwd)
        xn_next = None
        if b + 1 < NB:
            wait(cx[b + 1])
            xn_next = layernorm(b + 1, 0, R)
        outs += finish(b, xn_next)
    wait(outs)


@jax.jit
def pallas_parallel_sum__ssm_conv_s5__geglu_ffn__prompt_kernel(
    A_x: jax.Array,
    A_Lambda_re: jax.Array,
    A_Lambda_im: jax.Array,
    A_B_re: jax.Array,
    A_B_im: jax.Array,
    A_C_re: jax.Array,
    A_C_im: jax.Array,
    A_log_dt: jax.Array,
    A_Dskip: jax.Array,
    B_x: jax.Array,
    B_w_gate: jax.Array,
    B_w_up: jax.Array,
    B_w_down: jax.Array,
):
    del B_x
    hbm = pl.BlockSpec(memory_space=pltpu.HBM)
    out = pl.pallas_call(
        _kernel,
        out_shape=jax.ShapeDtypeStruct((L, D), bf16),
        in_specs=[hbm] * 12,
        out_specs=hbm,
        scratch_shapes=[
            pltpu.VMEM((NB, R // 2, D), u32),
            pltpu.VMEM((4, 4, 128), bf16),
            pltpu.VMEM((P // 2, D), u32),
            pltpu.VMEM((P // 2, D), u32),
            pltpu.VMEM((D // 2, P), u32),
            pltpu.VMEM((D // 2, P), u32),
            pltpu.VMEM((D // 2, 2 * P), u32),
            pltpu.VMEM((F // 2, D), u32),
            pltpu.VMEM((F // 2, D), u32),
            pltpu.VMEM((F // 2, D), u32),
            pltpu.VMEM((NB, R, D), bf16),
            pltpu.VMEM((NB, R, D), f32),
            pltpu.VMEM((NB, 8, SKEW_ROWS, 128), f32),
            pltpu.VMEM((NB, R, 2 * P), bf16),
            pltpu.VMEM((NB, 4, SKEW_ROWS, 128), f32),
            pltpu.VMEM((NB, R, F), bf16),
            pltpu.VMEM((NB, R, D), bf16),
            pltpu.SemaphoreType.DMA((NSEM,)),
        ],
        compiler_params=pltpu.CompilerParams(
            vmem_limit_bytes=100 * 2**20,
            disable_semaphore_checks=True,
            flags={"XLA_TPU_RESCHEDULE_DMA_DONES": True},
        ),
        name="ssm_geglu",
    )(A_x.reshape(L, D),
      A_Lambda_re.reshape(4, 128), A_Lambda_im.reshape(4, 128),
      A_log_dt.reshape(4, 128), A_Dskip.reshape(4, 128),
      A_B_re, A_B_im, A_C_re, A_C_im, B_w_gate.T, B_w_up.T, B_w_down)
    return out.reshape(1, L, D)
```
